```python
import os as _os
_os.environ.setdefault("JAX_PLATFORMS", "cpu")
import jax
import jax.numpy as jnp

def _softmax(x, axis=-1):
    return jax.nn.softmax(x, axis=axis)
def _gelu(x):
    return jax.nn.gelu(x, approximate=True)
def _silu(x):
    return jax.nn.silu(x)
def _sigmoid(x):
    return jax.nn.sigmoid(x)
def _layernorm(x, axis=-1, eps=1e-5):
    m = jnp.mean(x, axis=axis, keepdims=True)
    v = jnp.var(x, axis=axis, keepdims=True)
    return (x - m) / jnp.sqrt(v + eps)
def _scatter_add(tgt, idx, src, axis=0):
    return tgt.at[idx].add(src)
def _segment_sum(src, seg, n):
    return jax.ops.segment_sum(src, seg, n)
class _Rng:
    def __init__(self, key):
        self._k = key
    def _next(self):
        self._k, sub = jax.random.split(self._k)
        return sub
    def normal(self, shape):
        return jax.random.normal(self._next(), shape, dtype=jnp.bfloat16)
    def randint(self, lo, hi, shape):
        return jax.random.randint(self._next(), shape, lo, hi, dtype=jnp.int32)
    def uniform(self, shape, lo=0.0, hi=1.0):
        return jax.random.uniform(self._next(), shape, jnp.bfloat16, lo, hi)
    def permutation(self, n):
        return jax.random.permutation(self._next(), n)


kernel_name = 'concat_heads__ssm_conv_s4__linear_attn_block__prompt'

def setup_inputs():
    _rng = _Rng(jax.random.key(int.from_bytes(__import__("os").urandom(4), "little")))
    _w = (lambda a: (lambda t: t.astype(jnp.bfloat16) if jnp.issubdtype(t.dtype, jnp.floating) else t)(jnp.asarray(a)))
    def _A_setup():
        B, L, D, N = 1, 2048, 512, 128
        A_re = -jnp.exp((lambda *s: _rng.normal(s) * 0.1)(D, N))
        A_im = jnp.pi * (lambda *s: _rng.normal(s) * 0.1)(D, N)
        B_re = (lambda *s: _rng.normal(s) * 0.1)(D, N)
        B_im = (lambda *s: _rng.normal(s) * 0.1)(D, N)
        C_re = (lambda *s: _rng.normal(s) * 0.1)(D, N)
        C_im = (lambda *s: _rng.normal(s) * 0.1)(D, N)
        log_dt = (lambda *s: _rng.normal(s) * 0.1)(D) * 0.5 - 4.0
        Dskip = (lambda *s: _rng.normal(s) * 0.05)(D)
        return {
            "u": _w((lambda *s: _rng.normal(s) * 0.05)(B, L, D)),
            "A_re": _w(A_re),
            "A_im": _w(A_im),
            "B_re": _w(B_re),
            "B_im": _w(B_im),
            "C_re": _w(C_re),
            "C_im": _w(C_im),
            "log_dt": _w(log_dt),
            "Dskip": _w(Dskip),
        }
    _A_in = _A_setup()

    def _B_setup():
        B, S, D = 1, 2048, 512
        return {
            "x": _w((lambda *s: _rng.normal(s) * 0.05)(B, S, D)),
            "wqkv": _w((lambda *s: _rng.normal(s) * 0.4)(D, 3 * D)),
            "wo": _w((lambda *s: _rng.normal(s) * 0.05)(D, D)),
        }
    _B_in = _B_setup()

    return {
        "A_u": _A_in["u"],
        "A_A_re": _A_in["A_re"],
        "A_A_im": _A_in["A_im"],
        "A_B_re": _A_in["B_re"],
        "A_B_im": _A_in["B_im"],
        "A_C_re": _A_in["C_re"],
        "A_C_im": _A_in["C_im"],
        "A_log_dt": _A_in["log_dt"],
        "A_Dskip": _A_in["Dskip"],
        "B_x": _B_in["x"],
        "B_wqkv": _B_in["wqkv"],
        "B_wo": _B_in["wo"],
    }

def reference(A_u, A_A_re, A_A_im, A_B_re, A_B_im, A_C_re, A_C_im, A_log_dt, A_Dskip, B_x, B_wqkv, B_wo):
    def _A_ref(u, A_re, A_im, B_re, B_im, C_re, C_im, log_dt, Dskip):
        Bsz, L, D = u.shape
        dt = jnp.exp(log_dt)[:, None]
        A = A_re + 1j * A_im
        Bc = B_re + 1j * B_im
        Cc = C_re + 1j * C_im
        logdA = dt * A
        dB = dt * Bc
        l = (lambda x, dt: x.astype(dt))(jnp.arange(L), A_re.dtype)
        P = jnp.exp(logdA[:, :, None] * l[None, None, :])
        K = jnp.einsum("dn,dnl,dn->dl", Cc, P, dB).real
        L2 = 2 * L
        Kp = jnp.pad(K, ((0, 0), (0, L)))
        up = (lambda x, *d: x.transpose(*d))(u, 0, 2, 1)
        up = jnp.pad(up, ((0, 0), (0, 0), (0, L)))
        Kf = (lambda x, axes=(-2,-1): jnp.fft.rfft2(x.astype(jnp.float32), axes=axes))(Kp[:, None, :], axes=(-2, -1))
        Uf = (lambda x, axes=(-2,-1): jnp.fft.rfft2(x.astype(jnp.float32), axes=axes))(up[:, :, None, :], axes=(-2, -1))
        Yf = Uf * Kf[None, :, :, :]
        y = (lambda x, s, axes=(-2,-1): jnp.fft.irfft2(x, s=s, axes=axes).astype(jnp.bfloat16))(Yf, (1, L2), axes=(-2, -1))[:, :, 0, :L]
        y = (lambda x, *d: x.transpose(*d))(y, 0, 2, 1) + u * Dskip[None, None, :]
        return y

    def _B_ref(x, wqkv, wo):
        B, S, D = x.shape
        H = 32; Dh = D // H
        qkv = (lambda x, *d: x.transpose(*d))((x @ wqkv).reshape(B, S, 3, H, Dh), 2, 0, 3, 1, 4)
        q, k, v = qkv[0], qkv[1], qkv[2]
        phi = lambda t: jnp.where(t > 0, t + 1, jnp.exp(t)) + 1e-6
        pq, pk = phi(q), phi(k)
        kv = jnp.einsum("bhsd,bhse->bhde", pk, v)
        z = jnp.einsum("bhsd->bhd", pk)
        num = jnp.einsum("bhqd,bhde->bhqe", pq, kv)
        den = jnp.einsum("bhqd,bhd->bhq", pq, z)[..., None] + 1e-6
        o = num / den
        return (lambda x, *d: x.transpose(*d))(o, 0, 2, 1, 3).reshape(B, S, D) @ wo

    a = _A_ref(A_u, A_A_re, A_A_im, A_B_re, A_B_im, A_C_re, A_C_im, A_log_dt, A_Dskip)
    b = _B_ref(B_x, B_wqkv, B_wo)
    return jnp.concatenate([a, b], axis=-1)
```

```python
import numpy as np
import jax
import jax.numpy as jnp
import jax.experimental.pallas as pl
import jax.experimental.pallas.tpu as pltpu

F32 = jnp.float32
BF16 = jnp.bfloat16

L = 2048
D = 512
N = 128
C = 128
NC = L // C
NG = D // 8
H = 32
DH = D // H


def _bf16_round_int(l):
    u = np.asarray(l, np.float32).view(np.uint32)
    r = (u + 0x7FFF + ((u >> 16) & 1)) & 0xFFFF0000
    return r.astype(np.uint32).view(np.float32).astype(np.int64)


_BASES = (
    [q for q in range(8)]
    + [128 + q for q in range(8)]
    + [256 + 128 * k + 2 * q for k in range(2) for q in range(4)]
    + [512 + 128 * k + 4 * q for k in range(4) for q in range(2)]
    + [1024 + 128 * k for k in range(8)]
    + [2048]
)
NR = len(_BASES)
NZ = 6


def _tables():
    loc = {}
    for r, b in enumerate(_BASES):
        p, q = divmod(r, 8)
        for c in range(16):
            loc.setdefault(b + 8 * c, (p, (8 * c + 7 + q) % 128))
    theta = 2 * np.pi * (np.arange(C) + 0.5) / (2 * C)

    def col(b):
        return np.concatenate([np.cos(theta * b), -np.sin(theta * b)])

    fwd = np.stack([col(b) for b in range(C)], axis=1)
    g = {}
    for k in range(NC):
        for b in range(C):
            v = int(_bf16_round_int(C * k + b))
            p, lane = loc[v]
            g.setdefault((k, p), np.zeros((2 * C, C)))[:, lane] += col(b)
    ang = np.outer(np.arange(C), theta)
    inv = np.concatenate([np.cos(ang), -np.sin(ang)], axis=1) / C
    perm = np.array([part * C + 8 * rb + r for rb in range(C // 8) for part in range(2)
                     for r in range(8)])
    plan = []
    mats = []
    for k in range(NC):
        ps = sorted(p for (kk, p) in g if kk == k)
        assert ps == list(range(ps[0], ps[0] + len(ps)))
        plan.append((ps[0], len(ps), len(mats)))
        for p in ps:
            mats.append(g[(k, p)][perm])
    gmat = np.stack(mats)
    inv = inv[:, perm]
    inv = np.stack([inv[:, :C], inv[:, C:]])
    return fwd[perm], inv, gmat, tuple(plan)


_FWD, _INV, _GMAT, _GPLAN = _tables()
NGM = _GMAT.shape[0]


def _cmul(a, b):
    return (a[0] * b[0] - a[1] * b[1], a[0] * b[1] + a[1] * b[0])


def _csq(a):
    return (a[0] * a[0] - a[1] * a[1], 2.0 * (a[0] * a[1]))


def _rev8(x, sub):
    x = pltpu.roll(x, 4, 0)
    x = jnp.where((sub & 2) != 0, pltpu.roll(x, 2, 0), pltpu.roll(x, 6, 0))
    x = jnp.where((sub & 1) != 0, pltpu.roll(x, 1, 0), pltpu.roll(x, 7, 0))
    return x


def _gen_tables(zr, zi, cbr, cbi):
    sub = jax.lax.broadcasted_iota(jnp.int32, (8, 128), 0)
    z1 = (zr, zi)
    z2 = _csq(z1); z4 = _csq(z2); z8 = _csq(z4)
    z16 = _csq(z8); z32 = _csq(z16); z64 = _csq(z32)
    z128 = _csq(z64); z256 = _csq(z128); z512 = _csq(z256); z1024 = _csq(z512)
    q8 = (_rev8(z8[0], sub), -_rev8(z8[1], sub))
    one = (jnp.ones_like(zr), jnp.zeros_like(zr))
    q16 = _csq(q8); q32 = _csq(q16); q64 = _csq(q32)
    Q = [one, q8, q16, _cmul(q16, q8)]
    Q += [q32] + [_cmul(q32, Q[i]) for i in range(1, 4)]
    Q += [q64] + [_cmul(q64, Q[i]) for i in range(1, 8)]
    p0 = (cbr, cbi)
    P0 = [p0, _cmul(p0, z1)]
    P0 += [_cmul(P0[0], z2), _cmul(P0[1], z2)]
    P0 += [_cmul(p, z4) for p in P0]
    P1 = [_cmul(p, z128) for p in P0]
    a = _cmul(p0, z256)
    a2 = _cmul(a, z2)
    R1 = [a, a2, _cmul(a, z4), _cmul(a2, z4)]
    R1 += [_cmul(p, z128) for p in R1]
    b0 = _cmul(p0, z512)
    b0 = [b0, _cmul(b0, z4)]
    b1 = [_cmul(p, z128) for p in b0]
    b2 = [_cmul(p, z256) for p in b0]
    b3 = [_cmul(p, z128) for p in b2]
    R2 = b0 + b1 + b2 + b3
    c0 = _cmul(p0, z1024)
    R3 = [c0, _cmul(c0, z128)]
    R3 += [_cmul(p, z256) for p in R3]
    R3 += [_cmul(p, z512) for p in R3]
    last = _cmul(c0, z1024)
    P = P0 + P1 + R1 + R2 + R3 + [last]
    zero = jnp.zeros_like(zr)
    lr = jnp.concatenate([p[0] for p in P] + [zero], axis=0).astype(BF16)
    li = jnp.concatenate([p[1] for p in P] + [zero], axis=0).astype(BF16)
    rr = jnp.concatenate([q[0] for q in Q], axis=0).astype(BF16)
    ri = jnp.concatenate([q[1] for q in Q], axis=0).astype(BF16)
    return lr, li, rr, ri


U32 = jnp.uint32


def _ld(wref, *idx):
    *lead, rows = idx
    if rows is None:
        v = wref[tuple(lead) + (slice(None), slice(None))]
    else:
        start, size = rows
        if isinstance(start, int):
            rs = slice(start // 2, (start + size) // 2)
        else:
            rs = pl.ds(pl.multiple_of(start // 2, 8), size // 2)
        v = wref[tuple(lead) + (rs, slice(None))]
    return pltpu.bitcast(v, BF16)


def _st(bref, val, *idx):
    *lead, rows = idx
    if rows is None:
        bref[tuple(lead) + (slice(None), slice(None))] = val
    else:
        start, size = rows
        if isinstance(start, int):
            rs = slice(start, start + size)
        else:
            rs = pl.ds(pl.multiple_of(start, 16), size)
        bref[tuple(lead) + (rs, slice(None))] = val


def _cat(wref, idxs, rows=None):
    return jnp.concatenate([_ld(wref, i, rows) for i in idxs], axis=1)


def _kgen_matmul(lm, rm):
    lane = jax.lax.broadcasted_iota(jnp.int32, (8, 128), 1)
    lq = (lane + 1) & 7
    out = jax.lax.dot_general(lm, rm, (((1,), (1,)), ((), ())),
                              preferred_element_type=F32)
    zs = []
    for p in range(NZ):
        acc = None
        for q in range(8):
            r = 8 * p + q
            if r >= NR:
                break
            t = pltpu.roll(out[8 * r:8 * r + 8, :], q, 1, stride=1, stride_axis=0)
            acc = t if acc is None else jnp.where(lq == q, t, acc)
        zs.append(acc)
    return zs


def _phi(t):
    return jnp.where(t > 0, t + 1.0, jnp.exp(t)) + 1e-6


def _sincos(x):
    k = jnp.floor(x * 0.6366197723675814 + 0.5)
    r = ((x - k * 1.5703125) - k * 4.837512969970703125e-4) - k * 7.54978995489188216e-8
    r2 = r * r
    s = r + r * r2 * (-1.6666654611e-1 + r2 * (8.3321608736e-3 + r2 * -1.9515295891e-4))
    c = 1.0 - 0.5 * r2 + r2 * r2 * (4.166664568298827e-2
                                    + r2 * (-1.388731625493765e-3 + r2 * 2.443315711809948e-5))
    q = k.astype(jnp.int32)
    swap = (q & 1) != 0
    so = jnp.where(swap, c, s)
    co = jnp.where(swap, s, c)
    so = jnp.where((q & 2) != 0, -so, so)
    co = jnp.where(((q + 1) & 2) != 0, -co, co)
    return so, co


NT = D // 128
N4 = 3
N3 = 5
PACE4 = 0
PACE3 = 1
OB = 4
GB = 8
RB = 256


def _kernel(are_ref, aim_ref, bre_ref, bim_ref, cre_ref, cim_ref, ldt_ref, dsk_ref,
            fwd_ref, inv_ref,
            u_hbm, x_hbm, wqkv_hbm, wo_hbm, g_hbm,
            out_hbm,
            u_v, x_v, wqkv_v, wo_v, g_v, out_v,
            ar_s, ai_s, cbr_s, cbi_s,
            la_s, ra_s, lb_s, rb_s,
            z_s, zb_s, kf_s, uf_s, vt_s, y_s,
            wkt_s, s1_s, zacc_s, pq_s, m_s, zf_s, zm_s, pn_s,
            in_sem, out_sem):
    (u_w, x_w, wqkv_w, wo_w, g_w, la_w, ra_w, lb_w, rb_w, zb_w, wkt_w, pq_w, m_w, zf_w,
     fwd_w, inv_w, pn_w) = [r.bitcast(U32) for r in (
         u_v, x_v, wqkv_v, wo_v, g_v, la_s, ra_s, lb_s, rb_s, zb_s, wkt_s, pq_s, m_s, zf_s,
         fwd_ref, inv_ref, pn_s)]

    def slab_copies(src, dst, n, sem):
        return [pltpu.make_async_copy(src.at[:, 128 * t:128 * (t + 1)], dst.at[t], sem)
                for t in range(n)]

    cp_g = [pltpu.make_async_copy(g_hbm, g_v, in_sem.at[0])]
    cp_u = slab_copies(u_hbm.at[0], u_v, NT, in_sem.at[1])
    cp_x = slab_copies(x_hbm.at[0], x_v, NT, in_sem.at[2])
    cp_w = slab_copies(wqkv_hbm, wqkv_v, 3 * NT, in_sem.at[3])
    cp_o = slab_copies(wo_hbm, wo_v, NT, in_sem.at[4])
    for cp in cp_g + cp_u + cp_x + cp_w + cp_o:
        cp.start()

    def wait_all(cps):
        for cp in cps:
            cp.wait()

    dt_row = jnp.exp(ldt_ref[...].astype(F32)).astype(BF16).astype(F32)
    dt = jnp.broadcast_to(dt_row, (N, D)).T
    ar_s[...] = dt * are_ref[...].astype(F32)
    ai_s[...] = dt * aim_ref[...].astype(F32)
    dbr = dt * bre_ref[...].astype(F32)
    dbi = dt * bim_ref[...].astype(F32)
    cr = cre_ref[...].astype(F32)
    ci = cim_ref[...].astype(F32)
    cbr_s[...] = cr * dbr - ci * dbi
    cbi_s[...] = cr * dbi + ci * dbr
    s1_s[...] = jnp.zeros_like(s1_s)
    zacc_s[...] = jnp.zeros_like(zacc_s)

    def gen(g0, l_s, r_s):
        for b in range(GB):
            sl = pl.ds(pl.multiple_of((g0 + b) * 8, 8), 8)
            e = jnp.exp(ar_s[sl, :])
            sn, cs = _sincos(ai_s[sl, :])
            lr, li, rr, ri = _gen_tables(e * cs, e * sn, cbr_s[sl, :], cbi_s[sl, :])
            _st(l_s, lr, b, 0, None)
            _st(l_s, li, b, 1, None)
            _st(r_s, rr, b, 0, None)
            _st(r_s, ri, b, 1, None)

    def mm(g0, l_s, r_s):
        for b in range(GB):
            sl = pl.ds(pl.multiple_of((g0 + b) * 8, 8), 8)
            lm = jnp.concatenate([_ld(l_s, b, h, None) for h in range(2)], axis=1)
            rm = jnp.concatenate([_ld(r_s, b, h, None) for h in range(2)], axis=1)
            zs = _kgen_matmul(lm, rm)
            for p in range(NZ):
                z_s[p, sl, :] = zs[p]

    gen(0, la_s, ra_s)

    def p1_body(h, carry):
        g = 2 * GB * h
        mm(g, la_w, ra_w)
        gen(g + GB, lb_s, rb_s)
        mm(g + GB, lb_w, rb_w)
        gen(jnp.minimum(g + 2 * GB, NG - GB), la_s, ra_s)
        return carry

    with jax.named_scope('p1'):
        jax.lax.fori_loop(0, NG // (2 * GB), p1_body, 0)

    srow = jax.lax.broadcasted_iota(jnp.int32, (8, 128), 0)
    sgn = jnp.where((srow & 1) == 0, 1.0, -1.0).astype(F32)
    zm_s[...] = jnp.zeros_like(zm_s)

    def _bits(v):
        return pltpu.bitcast(v, jnp.int32)

    def _gate(v, g):
        return pltpu.bitcast(_bits(v) | g, F32)

    def conv_pos(t, rb, vt, g, pace):
        zm = zm_s[...]
        pr = pi_ = None
        for j in range(NC):
            ur = uf_s[t, j, rb, 0]
            ui = uf_s[t, j, rb, 1]
            if j == 0:
                vr, vi = ur, ui
            else:
                vr = ur - sgn * pi_
                vi = ui + sgn * pr
            vt[j, 0] = vr
            vt[j, 1] = vi
            vt[j, 2] = vr + vi
            pr, pi_ = ur, ui
        for a in range(NC // OB):
            i0 = OB * a
            t1 = [None] * OB
            t2 = [None] * OB
            t3 = [None] * OB
            kw = {}
            for j in range(i0 + OB):
                vr = _gate(vt[j, 0], g)
                vi = _gate(vt[j, 1], g)
                vs = _gate(vt[j, 2], g)
                for ii in range(OB):
                    k = i0 + ii - j
                    if k < 0:
                        continue
                    if k not in kw:
                        kw[k] = (kf_s[t, k, rb, 0], kf_s[t, k, rb, 1], kf_s[t, k, rb, 2])
                    kr, kd, ks = kw[k]
                    a1 = kr * vs
                    a2 = vr * kd
                    a3 = vi * ks
                    t1[ii] = a1 if t1[ii] is None else t1[ii] + a1
                    t2[ii] = a2 if t2[ii] is None else t2[ii] + a2
                    t3[ii] = a3 if t3[ii] is None else t3[ii] + a3
                g = _bits(t1[OB - 1]) & zm
                for _ in range(pace):
                    g = (g | _bits(t2[OB - 1])) & zm
            for ii in range(OB):
                y_s[t, i0 + ii, rb, 0] = t1[ii] - t3[ii]
                y_s[t, i0 + ii, rb, 1] = t1[ii] + t2[ii]
        return g

    for p in range(NZ):
        _st(zb_s, z_s[p].astype(BF16), p, None)
    wait_all(cp_g)
    wait_all(cp_u)
    fwd = _ld(fwd_w, None)

    with jax.named_scope('p2'):
        for k in range(NC):
            p0, np_, gi = _GPLAN[k]
            acc = jax.lax.dot_general(
                _cat(g_w, range(gi, gi + np_)), _cat(zb_w, range(p0, p0 + np_)),
                (((1,), (1,)), ((), ())), preferred_element_type=F32)
            acc = acc.reshape(C // 8, 2, 8, D)
            kr = acc[:, 0]
            ki = acc[:, 1]
            kd = ki - kr
            ks = kr + ki
            for t in range(NT):
                cs = slice(128 * t, 128 * (t + 1))
                kf_s[t, k, :, 0] = kr[:, :, cs]
                kf_s[t, k, :, 1] = kd[:, :, cs]
                kf_s[t, k, :, 2] = ks[:, :, cs]
        for j in range(NC):
            uf = jnp.dot(fwd, _cat(u_w, range(NT), (C * j, C)), preferred_element_type=F32)
            uf = uf.reshape(C // 8, 2, 8, D)
            for t in range(NT):
                uf_s[t, j] = uf[:, :, :, 128 * t:128 * (t + 1)]

    wait_all(cp_w)
    wkt = _cat(wqkv_w, range(NT, 2 * NT)).astype(F32).T.astype(BF16)
    for t in range(NT):
        _st(wkt_s, wkt[:, 128 * t:128 * (t + 1)], t, None)
    wait_all(cp_x)

    n3 = L // RB

    def p3_body(it, carry):
        rows = (it * RB, RB)
        xt = [_ld(x_w, t, rows) for t in range(NT)]
        xb = jnp.concatenate(xt, axis=1)

        def qpiece(t):
            q = jnp.dot(xb, _ld(wqkv_w, t, None), preferred_element_type=F32)
            _st(pq_s, _phi(q).astype(BF16), t, rows)

        def kpiece(c):
            kt = jax.lax.dot_general(_cat(wkt_w, range(NT)), xb[128 * c:128 * (c + 1), :],
                                     (((1,), (1,)), ((), ())),
                                     preferred_element_type=F32)
            return _phi(kt)

        def spiece(pk, t):
            cs = slice(128 * t, 128 * (t + 1))
            s1_s[:, cs] += jnp.dot(pk, xt[t], preferred_element_type=F32)

        k0 = kpiece(0)
        k1 = kpiece(1)
        zacc_s[...] += k0 + k1
        pk = jnp.concatenate([k0.astype(BF16), k1.astype(BF16)], axis=1)
        for t in range(4):
            qpiece(t)
        for t in range(4):
            spiece(pk, t)
        g = zm_s[...]
        for sidx in range(N3):
            e = it * N3 + sidx
            g = conv_pos(e // (C // 8), e % (C // 8), vt_s.at[sidx], g, PACE3)
        return carry

    with jax.named_scope('p3'):
        jax.lax.fori_loop(0, n3, p3_body, 0)

    wait_all(cp_o)
    zcol = jnp.sum(zacc_s[...], axis=1, keepdims=True)
    ri = jax.lax.broadcasted_iota(jnp.int32, (128, 128), 0)
    ci_ = jax.lax.broadcasted_iota(jnp.int32, (128, 128), 1)
    same_head = (ri // DH) == (ci_ // DH)
    for g in range(D // 128):
        gs = slice(128 * g, 128 * (g + 1))
        kv = jnp.dot(s1_s[gs, :].astype(BF16), _ld(wqkv_w, 2 * NT + g, None),
                     preferred_element_type=F32)
        kv = jnp.where(same_head, kv, 0.0).astype(BF16)
        for t in range(NT):
            mt = jnp.dot(kv, _ld(wo_w, t, (128 * g, 128)), preferred_element_type=F32)
            _st(m_s, mt.astype(BF16), t, (128 * g, 128))
        _st(zf_s, jnp.where(same_head, zcol[gs, :], 0.0).astype(BF16), g, None)

    inv = _cat(inv_w, range(2))
    dsk = dsk_ref[...].astype(F32)
    cpb = RB // C

    def normalise(blk, g):
        pg = _ld(pq_w, g, (blk * RB, RB))
        den = jnp.dot(pg, _ld(zf_w, g, None), preferred_element_type=F32) + 1e-6
        r = pl.reciprocal(den, approx=True)
        r = r * (2.0 - den * r)
        _st(pn_s, (pg.astype(F32) * r).astype(BF16), g, (blk * RB, RB))

    for g in range(NT):
        normalise(0, g)

    def p4_body(it, carry):
        rows = pl.ds(pl.multiple_of(it * RB, RB), RB)
        pqn = _cat(pn_w, range(NT), (it * RB, RB))
        for t in range(NT):
            normalise(jnp.minimum(it + 1, n3 - 1), t)
            ob = jnp.dot(pqn, _ld(m_w, t, None), preferred_element_type=F32)
            out_v[rows, D + 128 * t:D + 128 * (t + 1)] = ob.astype(BF16)
        pltpu.make_async_copy(out_v.at[rows, D:2 * D], out_hbm.at[0, rows, D:2 * D],
                              out_sem.at[0, it]).start()
        g = zm_s[...]
        for sidx in range(N4):
            e = n3 * N3 + it * N4 + sidx
            g = conv_pos(e // (C // 8), e % (C // 8), vt_s.at[sidx], g, PACE4)
        return carry

    with jax.named_scope('p4'):
        jax.lax.fori_loop(0, n3, p4_body, 0)

    def p5_body(it, carry):
        rows = pl.ds(pl.multiple_of(it * RB, RB), RB)
        for c in range(cpb):
            crow = pl.ds(pl.multiple_of(it * RB + c * C, C), C)
            for t in range(NT):
                yf = y_s[t, it * cpb + c].reshape(2 * C, 128).astype(BF16)
                ya = jnp.dot(inv, yf, preferred_element_type=F32)
                ub = _ld(u_w, t, (it * RB + c * C, C)).astype(F32)
                ya = ya + ub * dsk[:, 128 * t:128 * (t + 1)]
                out_v[crow, 128 * t:128 * (t + 1)] = ya.astype(BF16)
        pltpu.make_async_copy(out_v.at[rows, 0:D], out_hbm.at[0, rows, 0:D],
                              out_sem.at[1, it]).start()
        return carry

    with jax.named_scope('p5'):
        jax.lax.fori_loop(0, n3, p5_body, 0)

    for h in range(2):
        for it in range(n3):
            rows = pl.ds(it * RB, RB)
            cols = slice(h * D, h * D + D) if h == 0 else slice(0, D)
            cols = slice(D, 2 * D) if h == 0 else slice(0, D)
            pltpu.make_async_copy(out_v.at[rows, cols], out_hbm.at[0, rows, cols],
                                  out_sem.at[h, it]).wait()


@jax.jit
def pallas_concat_heads__ssm_conv_s4__linear_attn_block__prompt_kernel(
    A_u: jax.Array,
    A_A_re: jax.Array,
    A_A_im: jax.Array,
    A_B_re: jax.Array,
    A_B_im: jax.Array,
    A_C_re: jax.Array,
    A_C_im: jax.Array,
    A_log_dt: jax.Array,
    A_Dskip: jax.Array,
    B_x: jax.Array,
    B_wqkv: jax.Array,
    B_wo: jax.Array,
):
    vmem = pl.BlockSpec(memory_space=pltpu.VMEM)
    hbm = pl.BlockSpec(memory_space=pl.ANY)
    npos = max(N3, N4)
    assert (L // RB) * (N3 + N4) == NT * (C // 8)
    scratch = [
        pltpu.VMEM((NT, L, 128), BF16),
        pltpu.VMEM((NT, L, 128), BF16),
        pltpu.VMEM((3 * NT, D, 128), BF16),
        pltpu.VMEM((NT, D, 128), BF16),
        pltpu.VMEM((NGM, 2 * C, C), BF16),
        pltpu.VMEM((L, 2 * D), BF16),
        pltpu.VMEM((D, N), F32),
        pltpu.VMEM((D, N), F32),
        pltpu.VMEM((D, N), F32),
        pltpu.VMEM((D, N), F32),
        pltpu.VMEM((GB, 2, 336, 128), BF16),
        pltpu.VMEM((GB, 2, 128, 128), BF16),
        pltpu.VMEM((GB, 2, 336, 128), BF16),
        pltpu.VMEM((GB, 2, 128, 128), BF16),
        pltpu.VMEM((NZ, D, 128), F32),
        pltpu.VMEM((NZ, D, 128), BF16),
        pltpu.VMEM((NT, NC, C // 8, 3, 8, 128), F32),
        pltpu.VMEM((NT, NC, C // 8, 2, 8, 128), F32),
        pltpu.VMEM((npos, NC, 3, 8, 128), F32),
        pltpu.VMEM((NT, NC, C // 8, 2, 8, 128), F32),
        pltpu.VMEM((NT, D, 128), BF16),
        pltpu.VMEM((D, D), F32),
        pltpu.VMEM((D, 128), F32),
        pltpu.VMEM((NT, L, 128), BF16),
        pltpu.VMEM((NT, D, 128), BF16),
        pltpu.VMEM((D // 128, 128, 128), BF16),
        pltpu.VMEM((8, 128), jnp.int32),
        pltpu.VMEM((NT, L, 128), BF16),
        pltpu.SemaphoreType.DMA((5,)),
        pltpu.SemaphoreType.DMA((2, L // RB)),
    ]
    return pl.pallas_call(
        _kernel,
        out_shape=jax.ShapeDtypeStruct((1, L, 2 * D), BF16),
        in_specs=[vmem] * 10 + [hbm] * 5,
        out_specs=hbm,
        scratch_shapes=scratch,
        compiler_params=pltpu.CompilerParams(vmem_limit_bytes=100 * 1024 * 1024),
    )(
        A_A_re, A_A_im, A_B_re, A_B_im, A_C_re, A_C_im,
        A_log_dt.reshape(1, D), A_Dskip.reshape(1, D),
        jnp.asarray(_FWD, BF16), jnp.asarray(_INV, BF16),
        A_u, B_x, B_wqkv, B_wo, jnp.asarray(_GMAT, BF16),
    )
```

```python
import numpy as np
import jax
import jax.numpy as jnp
import jax.experimental.pallas as pl
import jax.experimental.pallas.tpu as pltpu

F32 = jnp.float32
BF16 = jnp.bfloat16

L = 2048
D = 512
N = 128
C = 128
NC = L // C
NG = D // 8
H = 32
DH = D // H


def _bf16_round_int(l):
    u = np.asarray(l, np.float32).view(np.uint32)
    r = (u + 0x7FFF + ((u >> 16) & 1)) & 0xFFFF0000
    return r.astype(np.uint32).view(np.float32).astype(np.int64)


_BASES = (
    [q for q in range(8)]
    + [128 + q for q in range(8)]
    + [256 + 128 * k + 2 * q for k in range(2) for q in range(4)]
    + [512 + 128 * k + 4 * q for k in range(4) for q in range(2)]
    + [1024 + 128 * k for k in range(8)]
    + [2048]
)
NR = len(_BASES)
NZ = 6


def _tables():
    loc = {}
    for r, b in enumerate(_BASES):
        p, q = divmod(r, 8)
        for c in range(16):
            loc.setdefault(b + 8 * c, (p, (8 * c + 7 + q) % 128))
    theta = 2 * np.pi * (np.arange(C) + 0.5) / (2 * C)

    def col(b):
        return np.concatenate([np.cos(theta * b), -np.sin(theta * b)])

    fwd = np.stack([col(b) for b in range(C)], axis=1)
    g = {}
    for k in range(NC):
        for b in range(C):
            v = int(_bf16_round_int(C * k + b))
            p, lane = loc[v]
            g.setdefault((k, p), np.zeros((2 * C, C)))[:, lane] += col(b)
    ang = np.outer(np.arange(C), theta)
    inv = np.concatenate([np.cos(ang), -np.sin(ang)], axis=1) / C
    perm = np.array([part * C + 8 * rb + r for rb in range(C // 8) for part in range(2)
                     for r in range(8)])
    plan = []
    mats = []
    for k in range(NC):
        ps = sorted(p for (kk, p) in g if kk == k)
        assert ps == list(range(ps[0], ps[0] + len(ps)))
        plan.append((ps[0], len(ps), len(mats)))
        for p in ps:
            mats.append(g[(k, p)][perm])
    gmat = np.stack(mats)
    inv = inv[:, perm]
    inv = np.stack([inv[:, :C], inv[:, C:]])
    return fwd[perm], inv, gmat, tuple(plan)


_FWD, _INV, _GMAT, _GPLAN = _tables()
NGM = _GMAT.shape[0]


def _cmul(a, b):
    return (a[0] * b[0] - a[1] * b[1], a[0] * b[1] + a[1] * b[0])


def _csq(a):
    return (a[0] * a[0] - a[1] * a[1], 2.0 * (a[0] * a[1]))


def _rev8(x, sub):
    x = pltpu.roll(x, 4, 0)
    x = jnp.where((sub & 2) != 0, pltpu.roll(x, 2, 0), pltpu.roll(x, 6, 0))
    x = jnp.where((sub & 1) != 0, pltpu.roll(x, 1, 0), pltpu.roll(x, 7, 0))
    return x


def _gen_tables(zr, zi, cbr, cbi):
    sub = jax.lax.broadcasted_iota(jnp.int32, (8, 128), 0)
    z1 = (zr, zi)
    z2 = _csq(z1); z4 = _csq(z2); z8 = _csq(z4)
    z16 = _csq(z8); z32 = _csq(z16); z64 = _csq(z32)
    z128 = _csq(z64); z256 = _csq(z128); z512 = _csq(z256); z1024 = _csq(z512)
    q8 = (_rev8(z8[0], sub), -_rev8(z8[1], sub))
    one = (jnp.ones_like(zr), jnp.zeros_like(zr))
    q16 = _csq(q8); q32 = _csq(q16); q64 = _csq(q32)
    Q = [one, q8, q16, _cmul(q16, q8)]
    Q += [q32] + [_cmul(q32, Q[i]) for i in range(1, 4)]
    Q += [q64] + [_cmul(q64, Q[i]) for i in range(1, 8)]
    p0 = (cbr, cbi)
    P0 = [p0, _cmul(p0, z1)]
    P0 += [_cmul(P0[0], z2), _cmul(P0[1], z2)]
    P0 += [_cmul(p, z4) for p in P0]
    P1 = [_cmul(p, z128) for p in P0]
    a = _cmul(p0, z256)
    a2 = _cmul(a, z2)
    R1 = [a, a2, _cmul(a, z4), _cmul(a2, z4)]
    R1 += [_cmul(p, z128) for p in R1]
    b0 = _cmul(p0, z512)
    b0 = [b0, _cmul(b0, z4)]
    b1 = [_cmul(p, z128) for p in b0]
    b2 = [_cmul(p, z256) for p in b0]
    b3 = [_cmul(p, z128) for p in b2]
    R2 = b0 + b1 + b2 + b3
    c0 = _cmul(p0, z1024)
    R3 = [c0, _cmul(c0, z128)]
    R3 += [_cmul(p, z256) for p in R3]
    R3 += [_cmul(p, z512) for p in R3]
    last = c0[0] * z1024[0] - c0[1] * z1024[1]
    k_last = jnp.broadcast_to(jnp.sum(last, axis=1, keepdims=True), last.shape)
    P = P0 + P1 + R1 + R2 + R3
    lr = jnp.concatenate([p[0] for p in P], axis=0).astype(BF16)
    li = jnp.concatenate([p[1] for p in P], axis=0).astype(BF16)
    rr = jnp.concatenate([q[0] for q in Q], axis=0).astype(BF16)
    ri = jnp.concatenate([q[1] for q in Q], axis=0).astype(BF16)
    return lr, li, rr, ri, k_last


U32 = jnp.uint32


def _ld(wref, *idx):
    *lead, rows = idx
    if rows is None:
        v = wref[tuple(lead) + (slice(None), slice(None))]
    else:
        start, size = rows
        if isinstance(start, int):
            rs = slice(start // 2, (start + size) // 2)
        else:
            rs = pl.ds(pl.multiple_of(start // 2, 8), size // 2)
        v = wref[tuple(lead) + (rs, slice(None))]
    return pltpu.bitcast(v, BF16)


def _st(bref, val, *idx):
    *lead, rows = idx
    if rows is None:
        bref[tuple(lead) + (slice(None), slice(None))] = val
    else:
        start, size = rows
        if isinstance(start, int):
            rs = slice(start, start + size)
        else:
            rs = pl.ds(pl.multiple_of(start, 16), size)
        bref[tuple(lead) + (rs, slice(None))] = val


def _cat(wref, idxs, rows=None):
    return jnp.concatenate([_ld(wref, i, rows) for i in idxs], axis=1)


def _kgen_matmul(lm, rm):
    lane = jax.lax.broadcasted_iota(jnp.int32, (8, 128), 1)
    lq = (lane + 1) & 7
    out = jax.lax.dot_general(lm, rm, (((1,), (1,)), ((), ())),
                              preferred_element_type=F32)
    zs = []
    for p in range(NZ - 1):
        acc = None
        for q in range(8):
            r = 8 * p + q
            t = pltpu.roll(out[8 * r:8 * r + 8, :], q, 1, stride=1, stride_axis=0)
            acc = t if acc is None else jnp.where(lq == q, t, acc)
        zs.append(acc)
    return zs


def _phi(t):
    return jnp.where(t > 0, t + 1.0, jnp.exp(t)) + 1e-6


def _sincos(x):
    k = jnp.floor(x * 0.6366197723675814 + 0.5)
    r = ((x - k * 1.5703125) - k * 4.837512969970703125e-4) - k * 7.54978995489188216e-8
    r2 = r * r
    s = r + r * r2 * (-1.6666654611e-1 + r2 * (8.3321608736e-3 + r2 * -1.9515295891e-4))
    c = 1.0 - 0.5 * r2 + r2 * r2 * (4.166664568298827e-2
                                    + r2 * (-1.388731625493765e-3 + r2 * 2.443315711809948e-5))
    q = k.astype(jnp.int32)
    swap = (q & 1) != 0
    so = jnp.where(swap, c, s)
    co = jnp.where(swap, s, c)
    so = jnp.where((q & 2) != 0, -so, so)
    co = jnp.where(((q + 1) & 2) != 0, -co, co)
    return so, co


NT = D // 128
GB = 4
SPI = 8
RB = 512
OB = 4
N3 = 11
NKV = 4
N4 = 4
PACE3 = 1
PACEKV = 0
PACE4 = 1


def _kernel(ldt_hbm, dsk_hbm,
            are_hbm, aim_hbm, bre_hbm, bim_hbm, cre_hbm, cim_hbm,
            fwd_hbm, inv_hbm,
            u_hbm, x_hbm, wqkv_hbm, wo_hbm, g_hbm,
            out_hbm,
            ldt_ref, dsk_ref, par_v, fwd_v, inv_v,
            u_v, x_v, wqkv_v, wo_v, g_v, out_v,
            ar_s, ai_s, cbr_s, cbi_s,
            la_s, ra_s, lb_s, rb_s,
            z_s, zb_s, kf_s, uf_s, vt_s, y_s,
            wkt_s, s1_s, zacc_s, pq_s, m_s, zf_s, zm_s, pn_s,
            par_sem, in_sem, out_sem, osem_a):
    (u_w, x_w, wqkv_w, wo_w, g_w, la_w, ra_w, lb_w, rb_w, zb_w, wkt_w, pq_w, m_w, zf_w,
     fwd_w, inv_w, pn_w) = [r.bitcast(U32) for r in (
         u_v, x_v, wqkv_v, wo_v, g_v, la_s, ra_s, lb_s, rb_s, zb_s, wkt_s, pq_s, m_s, zf_s,
         fwd_v, inv_v, pn_s)]

    def slab_copies(src, dst, n, sem):
        return [pltpu.make_async_copy(src.at[:, 128 * t:128 * (t + 1)], dst.at[t], sem)
                for t in range(n)]

    pars = (are_hbm, aim_hbm, bre_hbm, bim_hbm, cre_hbm, cim_hbm)
    cp_p = [[pltpu.make_async_copy(src.at[128 * blk:128 * (blk + 1), :],
                                   par_v.at[a, 128 * blk:128 * (blk + 1), :], par_sem.at[blk])
             for a, src in enumerate(pars)] for blk in range(NT)]
    cp_p[0] = [pltpu.make_async_copy(ldt_hbm, ldt_ref, par_sem.at[0])] + cp_p[0]
    cp_g = [pltpu.make_async_copy(g_hbm, g_v, in_sem.at[0]),
            pltpu.make_async_copy(dsk_hbm, dsk_ref, in_sem.at[0]),
            pltpu.make_async_copy(fwd_hbm, fwd_v, in_sem.at[0]),
            pltpu.make_async_copy(inv_hbm, inv_v, in_sem.at[0])]
    cp_u = slab_copies(u_hbm.at[0], u_v, NT, in_sem.at[1])
    cp_x = slab_copies(x_hbm.at[0], x_v, NT, in_sem.at[2])
    cp_w = slab_copies(wqkv_hbm, wqkv_v, 3 * NT, in_sem.at[3])
    cp_o = slab_copies(wo_hbm, wo_v, NT, in_sem.at[4])
    for cp in sum(cp_p, []):
        cp.start()

    def wait_all(cps):
        for cp in cps:
            cp.wait()

    wait_all(cp_p[0])
    dt_row = jnp.exp(ldt_ref[...].astype(F32).reshape(1, D)).astype(BF16).astype(F32)

    def prep(blk):
        rs = slice(128 * blk, 128 * (blk + 1))
        dt = jnp.broadcast_to(dt_row[:, rs], (N, 128)).T
        are, aim, bre, bim, cr, ci = [par_v[a, rs, :].astype(F32) for a in range(6)]
        ar_s[rs, :] = dt * are
        ai_s[rs, :] = dt * aim
        dbr = dt * bre
        dbi = dt * bim
        cbr_s[rs, :] = cr * dbr - ci * dbi
        cbi_s[rs, :] = cr * dbi + ci * dbr

    prep(0)
    for blk in range(1, NT):
        wait_all(cp_p[blk])
    for cp in cp_g + cp_u + cp_x + cp_w + cp_o:
        cp.start()

    def grp(g):
        if isinstance(g, int):
            return slice(g * 8, g * 8 + 8)
        return pl.ds(pl.multiple_of(g * 8, 8), 8)

    def gen(g0, n, l_s, r_s):
        for b in range(n):
            sl = grp(g0 + b)
            e = jnp.exp(ar_s[sl, :])
            sn, cs = _sincos(ai_s[sl, :])
            lr, li, rr, ri, k_last = _gen_tables(e * cs, e * sn, cbr_s[sl, :], cbi_s[sl, :])
            z_s[NZ - 1, sl, :] = k_last
            _st(l_s, lr, b, 0, None)
            _st(l_s, li, b, 1, None)
            _st(r_s, rr, b, 0, None)
            _st(r_s, ri, b, 1, None)

    def mm(g0, n, l_s, r_s):
        for b in range(n):
            sl = grp(g0 + b)
            lm = jnp.concatenate([_ld(l_s, b, h, None) for h in range(2)], axis=1)
            rm = jnp.concatenate([_ld(r_s, b, h, None) for h in range(2)], axis=1)
            zs = _kgen_matmul(lm, rm)
            for p in range(NZ - 1):
                z_s[p, sl, :] = zs[p]

    gen(0, GB, la_s, ra_s)
    for blk in range(1, NT):
        prep(blk)
    n1 = NG // (GB * SPI)
    bufs = ((la_s, ra_s, la_w, ra_w), (lb_s, rb_s, lb_w, rb_w))

    def p1_body(h, carry):
        for i in range(SPI):
            g = (h * SPI + i) * GB
            cur, nxt = bufs[i % 2], bufs[(i + 1) % 2]
            mm(g, GB, cur[2], cur[3])
            gen(jnp.minimum(g + GB, NG - GB), GB, nxt[0], nxt[1])
        zr = pl.ds(pl.multiple_of(h * (D // n1), D // n1), D // n1)
        s1_s[zr, :] = jnp.zeros((D // n1, D), F32)
        return carry

    with jax.named_scope('p1'):
        jax.lax.fori_loop(0, n1, p1_body, 0)
    zacc_s[...] = jnp.zeros_like(zacc_s)

    srow = jax.lax.broadcasted_iota(jnp.int32, (8, 128), 0)
    sgn = jnp.where((srow & 1) == 0, 1.0, -1.0).astype(F32)
    zm_s[...] = jnp.zeros_like(zm_s)

    def _bits(v):
        return pltpu.bitcast(v, jnp.int32)

    def _gate(v, g):
        return pltpu.bitcast(_bits(v) | g, F32)

    def conv_pos(t, rb, vt, g, pace):
        zm = zm_s[...]
        pr = pi_ = None
        for j in range(NC):
            ur = uf_s[t, j, rb, 0]
            ui = uf_s[t, j, rb, 1]
            if j == 0:
                vr, vi = ur, ui
            else:
                vr = ur - sgn * pi_
                vi = ui + sgn * pr
            vt[j, 0] = vr
            vt[j, 1] = vi
            vt[j, 2] = vr + vi
            pr, pi_ = ur, ui
        for a in range(NC // OB):
            i0 = OB * a
            t1 = [None] * OB
            t2 = [None] * OB
            t3 = [None] * OB
            kw = {}
            for j in range(i0 + OB):
                vr = _gate(vt[j, 0], g)
                vi = _gate(vt[j, 1], g)
                vs = _gate(vt[j, 2], g)
                for ii in range(OB):
                    k = i0 + ii - j
                    if k < 0:
                        continue
                    if k not in kw:
                        kw[k] = (kf_s[t, k, rb, 0], kf_s[t, k, rb, 1], kf_s[t, k, rb, 2])
                    kr, kd, ks = kw[k]
                    a1 = kr * vs
                    a2 = vr * kd
                    a3 = vi * ks
                    t1[ii] = a1 if t1[ii] is None else t1[ii] + a1
                    t2[ii] = a2 if t2[ii] is None else t2[ii] + a2
                    t3[ii] = a3 if t3[ii] is None else t3[ii] + a3
                g = _bits(t1[OB - 1]) & zm
                for _ in range(pace):
                    g = (g | _bits(t2[OB - 1])) & zm
            for ii in range(OB):
                y_s[t, i0 + ii, rb, 0] = t1[ii] - t3[ii]
                y_s[t, i0 + ii, rb, 1] = t1[ii] + t2[ii]
        return g

    for p in range(NZ):
        _st(zb_s, z_s[p].astype(BF16), p, None)
    wait_all(cp_g)
    wait_all(cp_u)
    fwd = _ld(fwd_w, None)

    with jax.named_scope('p2'):
        for k in range(NC):
            p0, np_, gi = _GPLAN[k]
            acc = jax.lax.dot_general(
                _cat(g_w, range(gi, gi + np_)), _cat(zb_w, range(p0, p0 + np_)),
                (((1,), (1,)), ((), ())), preferred_element_type=F32)
            acc = acc.reshape(C // 8, 2, 8, D)
            kr = acc[:, 0]
            ki = acc[:, 1]
            kd = ki - kr
            ks = kr + ki
            for t in range(NT):
                cs = slice(128 * t, 128 * (t + 1))
                kf_s[t, k, :, 0] = kr[:, :, cs]
                kf_s[t, k, :, 1] = kd[:, :, cs]
                kf_s[t, k, :, 2] = ks[:, :, cs]
        wait_all(cp_w)
        wkt = _cat(wqkv_w, range(NT, 2 * NT)).astype(F32).T.astype(BF16)
        for t in range(NT):
            _st(wkt_s, wkt[:, 128 * t:128 * (t + 1)], t, None)
        for j in range(NC):
            uf = jnp.dot(fwd, _cat(u_w, range(NT), (C * j, C)), preferred_element_type=F32)
            uf = uf.reshape(C // 8, 2, 8, D)
            for t in range(NT):
                uf_s[t, j] = uf[:, :, :, 128 * t:128 * (t + 1)]

    wait_all(cp_x)

    n3 = L // RB

    def p3_body(it, carry):
        rows = (it * RB, RB)
        xt = [_ld(x_w, t, rows) for t in range(NT)]
        xb = jnp.concatenate(xt, axis=1)

        def qpiece(t):
            q = jnp.dot(xb, _ld(wqkv_w, t, None), preferred_element_type=F32)
            _st(pq_s, _phi(q).astype(BF16), t, rows)

        def kpiece(c):
            kt = jax.lax.dot_general(_cat(wkt_w, range(NT)), xb[128 * c:128 * (c + 1), :],
                                     (((1,), (1,)), ((), ())),
                                     preferred_element_type=F32)
            return _phi(kt)

        def spiece(pk, t):
            cs = slice(128 * t, 128 * (t + 1))
            s1_s[:, cs] += jnp.dot(pk, xt[t], preferred_element_type=F32)

        ks = [kpiece(c) for c in range(RB // 128)]
        za = ks[0]
        for kk in ks[1:]:
            za = za + kk
        zacc_s[...] += za
        pk = jnp.concatenate([kk.astype(BF16) for kk in ks], axis=1)
        for t in range(4):
            qpiece(t)
        for t in range(4):
            spiece(pk, t)
        g = zm_s[...]
        for sidx in range(N3):
            e = it * N3 + sidx
            g = conv_pos(e // (C // 8), e % (C // 8), vt_s.at[sidx], g, PACE3)
        return carry

    with jax.named_scope('p3'):
        jax.lax.fori_loop(0, n3, p3_body, 0)

    wait_all(cp_o)
    zcol = jnp.sum(zacc_s[...], axis=1, keepdims=True)
    ri = jax.lax.broadcasted_iota(jnp.int32, (128, 128), 0)
    ci_ = jax.lax.broadcasted_iota(jnp.int32, (128, 128), 1)
    same_head = (ri // DH) == (ci_ // DH)
    for g in range(D // 128):
        gs = slice(128 * g, 128 * (g + 1))
        kv = jnp.dot(s1_s[gs, :].astype(BF16), _ld(wqkv_w, 2 * NT + g, None),
                     preferred_element_type=F32)
        kv = jnp.where(same_head, kv, 0.0).astype(BF16)
        for t in range(NT):
            mt = jnp.dot(kv, _ld(wo_w, t, (128 * g, 128)), preferred_element_type=F32)
            _st(m_s, mt.astype(BF16), t, (128 * g, 128))
        _st(zf_s, jnp.where(same_head, zcol[gs, :], 0.0).astype(BF16), g, None)

    inv = _cat(inv_w, range(2))
    dsk = dsk_ref[...].astype(F32).reshape(1, D)
    cpb = RB // C

    def normalise(blk, g):
        pg = _ld(pq_w, g, (blk * RB, RB))
        den = jnp.dot(pg, _ld(zf_w, g, None), preferred_element_type=F32) + 1e-6
        den = jnp.minimum(den, 3.0e38)
        r = pl.reciprocal(den, approx=True)
        r = r * (2.0 - den * r)
        _st(pn_s, (pg.astype(F32) * r).astype(BF16), g, (blk * RB, RB))

    for g in range(NT):
        normalise(0, g)
    g = zm_s[...]
    for sidx in range(NKV):
        e = n3 * N3 + sidx
        g = conv_pos(e // (C // 8), e % (C // 8), vt_s.at[sidx], g, PACEKV)

    def p4_body(it, carry):
        rows = pl.ds(pl.multiple_of(it * RB, RB), RB)
        pqn = _cat(pn_w, range(NT), (it * RB, RB))
        for t in range(NT):
            normalise(jnp.minimum(it + 1, n3 - 1), t)
            ob = jnp.dot(pqn, _ld(m_w, t, None), preferred_element_type=F32)
            out_v[rows, D + 128 * t:D + 128 * (t + 1)] = ob.astype(BF16)
        pltpu.make_async_copy(out_v.at[rows, D:2 * D], out_hbm.at[0, rows, D:2 * D],
                              out_sem.at[it]).start()
        g = zm_s[...]
        for sidx in range(N4):
            e = n3 * N3 + NKV + it * N4 + sidx
            g = conv_pos(e // (C // 8), e % (C // 8), vt_s.at[sidx], g, PACE4)
        return carry

    with jax.named_scope('p4'):
        jax.lax.fori_loop(0, n3, p4_body, 0)

    def p5_body(it, carry):
        rows = pl.ds(pl.multiple_of(it * RB, RB), RB)
        for c in range(cpb):
            crow = pl.ds(pl.multiple_of(it * RB + c * C, C), C)
            for t in range(NT):
                yf = y_s[t, it * cpb + c].reshape(2 * C, 128).astype(BF16)
                ya = jnp.dot(inv, yf, preferred_element_type=F32)
                ub = _ld(u_w, t, (it * RB + c * C, C)).astype(F32)
                ya = ya + ub * dsk[:, 128 * t:128 * (t + 1)]
                out_v[crow, 128 * t:128 * (t + 1)] = ya.astype(BF16)
            pltpu.make_async_copy(out_v.at[crow, 0:D], out_hbm.at[0, crow, 0:D],
                                  osem_a.at[it * cpb + c]).start()
        return carry

    with jax.named_scope('p5'):
        jax.lax.fori_loop(0, n3, p5_body, 0)

    for it in range(n3):
        rows = pl.ds(it * RB, RB)
        pltpu.make_async_copy(out_v.at[rows, D:2 * D], out_hbm.at[0, rows, D:2 * D],
                              out_sem.at[it]).wait()
    for i in range(NC):
        rows = pl.ds(i * C, C)
        pltpu.make_async_copy(out_v.at[rows, 0:D], out_hbm.at[0, rows, 0:D],
                              osem_a.at[i]).wait()


@jax.jit
def pallas_concat_heads__ssm_conv_s4__linear_attn_block__prompt_kernel(
    A_u: jax.Array,
    A_A_re: jax.Array,
    A_A_im: jax.Array,
    A_B_re: jax.Array,
    A_B_im: jax.Array,
    A_C_re: jax.Array,
    A_C_im: jax.Array,
    A_log_dt: jax.Array,
    A_Dskip: jax.Array,
    B_x: jax.Array,
    B_wqkv: jax.Array,
    B_wo: jax.Array,
):
    hbm = pl.BlockSpec(memory_space=pl.ANY)
    npos = max(N3, N4, NKV)
    assert (L // RB) * (N3 + N4) + NKV == NT * (C // 8)
    scratch = [
        pltpu.VMEM((D,), BF16),
        pltpu.VMEM((D,), BF16),
        pltpu.VMEM((6, D, N), BF16),
        pltpu.VMEM((2 * C, C), BF16),
        pltpu.VMEM((2, C, C), BF16),
        pltpu.VMEM((NT, L, 128), BF16),
        pltpu.VMEM((NT, L, 128), BF16),
        pltpu.VMEM((3 * NT, D, 128), BF16),
        pltpu.VMEM((NT, D, 128), BF16),
        pltpu.VMEM((NGM, 2 * C, C), BF16),
        pltpu.VMEM((L, 2 * D), BF16),
        pltpu.VMEM((D, N), F32),
        pltpu.VMEM((D, N), F32),
        pltpu.VMEM((D, N), F32),
        pltpu.VMEM((D, N), F32),
        pltpu.VMEM((GB, 2, 320, 128), BF16),
        pltpu.VMEM((GB, 2, 128, 128), BF16),
        pltpu.VMEM((GB, 2, 320, 128), BF16),
        pltpu.VMEM((GB, 2, 128, 128), BF16),
        pltpu.VMEM((NZ, D, 128), F32),
        pltpu.VMEM((NZ, D, 128), BF16),
        pltpu.VMEM((NT, NC, C // 8, 3, 8, 128), F32),
        pltpu.VMEM((NT, NC, C // 8, 2, 8, 128), F32),
        pltpu.VMEM((npos, NC, 3, 8, 128), F32),
        pltpu.VMEM((NT, NC, C // 8, 2, 8, 128), F32),
        pltpu.VMEM((NT, D, 128), BF16),
        pltpu.VMEM((D, D), F32),
        pltpu.VMEM((D, 128), F32),
        pltpu.VMEM((NT, L, 128), BF16),
        pltpu.VMEM((NT, D, 128), BF16),
        pltpu.VMEM((D // 128, 128, 128), BF16),
        pltpu.VMEM((8, 128), jnp.int32),
        pltpu.VMEM((NT, L, 128), BF16),
        pltpu.SemaphoreType.DMA((NT,)),
        pltpu.SemaphoreType.DMA((5,)),
        pltpu.SemaphoreType.DMA((L // RB,)),
        pltpu.SemaphoreType.DMA((NC,)),
    ]
    return pl.pallas_call(
        _kernel,
        out_shape=jax.ShapeDtypeStruct((1, L, 2 * D), BF16),
        in_specs=[hbm] * 15,
        out_specs=hbm,
        scratch_shapes=scratch,
        compiler_params=pltpu.CompilerParams(vmem_limit_bytes=100 * 1024 * 1024),
    )(
        A_log_dt, A_Dskip,
        A_A_re, A_A_im, A_B_re, A_B_im, A_C_re, A_C_im,
        jnp.asarray(_FWD, BF16), jnp.asarray(_INV, BF16),
        A_u, B_x, B_wqkv, B_wo, jnp.asarray(_GMAT, BF16),
    )
```
